```python
import os as _os
_os.environ.setdefault("JAX_PLATFORMS", "cpu")
import jax
import jax.numpy as jnp

def _softmax(x, axis=-1):
    return jax.nn.softmax(x, axis=axis)
def _gelu(x):
    return jax.nn.gelu(x, approximate=True)
def _silu(x):
    return jax.nn.silu(x)
def _sigmoid(x):
    return jax.nn.sigmoid(x)
def _layernorm(x, axis=-1, eps=1e-5):
    m = jnp.mean(x, axis=axis, keepdims=True)
    v = jnp.var(x, axis=axis, keepdims=True)
    return (x - m) / jnp.sqrt(v + eps)
def _scatter_add(tgt, idx, src, axis=0):
    return tgt.at[idx].add(src)
def _segment_sum(src, seg, n):
    return jax.ops.segment_sum(src, seg, n)
class _Rng:
    def __init__(self, key):
        self._k = key
    def _next(self):
        self._k, sub = jax.random.split(self._k)
        return sub
    def normal(self, shape):
        return jax.random.normal(self._next(), shape, dtype=jnp.bfloat16)
    def randint(self, lo, hi, shape):
        return jax.random.randint(self._next(), shape, lo, hi, dtype=jnp.int32)
    def uniform(self, shape, lo=0.0, hi=1.0):
        return jax.random.uniform(self._next(), shape, jnp.bfloat16, lo, hi)
    def permutation(self, n):
        return jax.random.permutation(self._next(), n)


kernel_name = 'parallel_sum__ssm_conv_h3__dense_activation_silu__prompt'

def setup_inputs():
    _rng = _Rng(jax.random.key(int.from_bytes(__import__("os").urandom(4), "little")))
    _w = (lambda a: (lambda t: t.astype(jnp.bfloat16) if jnp.issubdtype(t.dtype, jnp.floating) else t)(jnp.asarray(a)))
    def _A_setup():
        B, S, D = 1, 2048, 448
        ks = 4
        return {
            "q": _w((lambda *s: _rng.normal(s) * 0.05)(B, S, D)),
            "k": _w((lambda *s: _rng.normal(s) * 0.2)(B, S, D)),
            "v": _w((lambda *s: _rng.normal(s) * 0.2)(B, S, D)),
            "shift_k": _w((lambda *s: _rng.normal(s) * 0.2)(D, ks) * 0.5),
            "ssm_k": _w((lambda *s: _rng.normal(s) * 0.2)(D, S) * (1.0 / S ** 0.5)),
            "ssm_D": _w((lambda *s: _rng.normal(s) * 0.2)(D)),
        }
    _A_in = _A_setup()

    def _B_setup():
        B, S, D, F = 1, 2048, 448, 1792
        return {
            "x": _w((lambda *s: _rng.normal(s) * 0.05)(B, S, D)),
            "w1": _w((lambda *s: _rng.normal(s) * 0.05)(D, F) * (D ** -0.5)),
            "w2": _w((lambda *s: _rng.normal(s) * 0.05)(F, D) * (F ** -0.5)),
        }
    _B_in = _B_setup()

    return {
        "A_q": _A_in["q"],
        "A_k": _A_in["k"],
        "A_v": _A_in["v"],
        "A_shift_k": _A_in["shift_k"],
        "A_ssm_k": _A_in["ssm_k"],
        "A_ssm_D": _A_in["ssm_D"],
        "B_x": _B_in["x"],
        "B_w1": _B_in["w1"],
        "B_w2": _B_in["w2"],
    }

def reference(A_q, A_k, A_v, A_shift_k, A_ssm_k, A_ssm_D, B_x, B_w1, B_w2):
    def _A_ref(q, k, v, shift_k, ssm_k, ssm_D):
        B, S, D = q.shape
        ks = shift_k.shape[-1]
        k_pad = jnp.pad(k, ((0, 0), (ks - 1, 0), (0, 0)))
        k_shift = jnp.zeros_like(k)
        for t in range(ks):
            k_shift = k_shift + k_pad[:, t:t + S, :] * shift_k[:, ks - 1 - t][None, None, :]
        kv = k_shift * v
        L = 2 * S
        kv_pad = jnp.pad(kv, ((0, 0), (0, S), (0, 0)))
        kf_pad = jnp.pad(ssm_k, ((0, 0), (0, S)))
        kv_f = (lambda x, axes=(-2,-1): jnp.fft.rfft2(x.astype(jnp.float32), axes=axes))(kv_pad[:, None, :, :], axes=(1, 2))
        kf_f = (lambda x, axes=(-2,-1): jnp.fft.rfft2(x.astype(jnp.float32), axes=axes))(kf_pad[:, None, :], axes=(1, 2))
        kf_f = (lambda x, *d: x.transpose(*d))(kf_f, 1, 2, 0)
        y_f = kv_f * kf_f[None, :, :, :]
        y = (lambda x, s, axes=(-2,-1): jnp.fft.irfft2(x, s=s, axes=axes).astype(jnp.bfloat16))(y_f, (1, L), axes=(1, 2))[:, 0, :S, :]
        y = y + kv * ssm_D[None, None, :]
        return q * y

    def _B_ref(x, w1, w2):
        h = jnp.einsum("bsd,df->bsf", x, w1)
        h = _silu(h)
        out = jnp.einsum("bsf,fd->bsd", h, w2)
        return out

    x = A_q
    xn = _layernorm(x, axis=-1)
    return x + _A_ref(xn, A_k, A_v, A_shift_k, A_ssm_k, A_ssm_D) + _B_ref(xn, B_w1, B_w2)
```

```python
import functools
import math

import jax
import jax.numpy as jnp
import jax.experimental.pallas as pl
import jax.experimental.pallas.tpu as pltpu

C = 128
RT = 16


def _split(x):
    hi = x.astype(jnp.bfloat16)
    lo = (x - hi.astype(jnp.float32)).astype(jnp.bfloat16)
    return hi, lo


def _kernel(q_ref, k_ref, v_ref, sk_ref, ssmk_ref, d_ref, w1_ref, w2_ref,
            o_ref,
            fhi_ref, flo_ref, ghi_ref, glo_ref, sgn_ref,
            kbuf_ref, hprev_ref, uf_ref, kf_ref, y_ref):
    a = pl.program_id(0)
    D = q_ref.shape[-1]

    @pl.when(a == 0)
    def _init():
        r = jax.lax.broadcasted_iota(jnp.int32, (2 * C, C), 0)
        n = jax.lax.broadcasted_iota(jnp.int32, (2 * C, C), 1)
        f = jnp.where(r > C, r - C, r)
        ang = ((f * n) % (2 * C)).astype(jnp.float32) * (math.pi / C)
        fm = jnp.where(r > C, -jnp.sin(ang), jnp.cos(ang))
        hi, lo = _split(fm)
        fhi_ref[...] = hi
        flo_ref[...] = lo
        b = jax.lax.broadcasted_iota(jnp.int32, (C, 2 * C), 0)
        c = jax.lax.broadcasted_iota(jnp.int32, (C, 2 * C), 1)
        f = jnp.where(c > C, c - C, c)
        ang = ((f * (b + C)) % (2 * C)).astype(jnp.float32) * (math.pi / C)
        scale = jnp.where((c == 0) | (c == C), 0.5 / C, 1.0 / C)
        gm = jnp.where(c > C, -jnp.sin(ang), jnp.cos(ang)) * scale
        hi, lo = _split(gm)
        ghi_ref[...] = hi
        glo_ref[...] = lo
        rr = jax.lax.broadcasted_iota(jnp.int32, (2 * C, D), 0)
        sgn_ref[...] = jnp.where(rr % 2 == 0, 1.0, -1.0).astype(jnp.float32)
        kbuf_ref[...] = jnp.zeros(kbuf_ref.shape, jnp.float32)
        hprev_ref[...] = jnp.zeros(hprev_ref.shape, jnp.float32)

    x = q_ref[0].astype(jnp.float32)
    mu = jnp.mean(x, axis=-1, keepdims=True)
    xc = x - mu
    var = jnp.mean(xc * xc, axis=-1, keepdims=True)
    xn = (xc * jax.lax.rsqrt(var + 1e-5)).astype(jnp.bfloat16)

    kbuf_ref[pl.ds(8, C), :] = k_ref[0].astype(jnp.float32)
    sk = sk_ref[...].astype(jnp.float32)
    ks = kbuf_ref[pl.ds(8, C), :] * sk[0:1, :]
    for j in range(1, sk.shape[0]):
        ks = ks + kbuf_ref[pl.ds(8 - j, C), :] * sk[j:j + 1, :]
    kbuf_ref[pl.ds(0, 8), :] = kbuf_ref[pl.ds(C, 8), :]
    kv = (ks.astype(jnp.bfloat16).astype(jnp.float32)
          * v_ref[0].astype(jnp.float32)).astype(jnp.bfloat16)

    fhi = fhi_ref[...]
    flo = flo_ref[...]
    h = (jnp.dot(fhi, kv, preferred_element_type=jnp.float32)
         + jnp.dot(flo, kv, preferred_element_type=jnp.float32))
    uf_ref[a] = hprev_ref[...] + sgn_ref[...] * h
    hprev_ref[...] = h
    kc = ssmk_ref[...]
    nt = (((1,), (1,)), ((), ()))
    kf_ref[a] = (jax.lax.dot_general(fhi, kc, nt, preferred_element_type=jnp.float32)
                 + jax.lax.dot_general(flo, kc, nt, preferred_element_type=jnp.float32))

    for rt in range(C // RT):
        rows_r = pl.ds(rt * RT, RT)
        rows_i = pl.ds(C + rt * RT, RT)

        def body(m, carry):
            A, B, Cc = carry
            kr = kf_ref[m, rows_r, :]
            ki = kf_ref[m, rows_i, :]
            ur = uf_ref[a - m, rows_r, :]
            ui = uf_ref[a - m, rows_i, :]
            return A + kr * ur, B + ki * ui, Cc + (kr * ui + ki * ur)

        z = jnp.zeros((RT, D), jnp.float32)
        A, B, Cc = jax.lax.fori_loop(0, a + 1, body, (z, z, z))
        if rt == 0:
            row0 = jax.lax.broadcasted_iota(jnp.int32, (RT, D), 0) == 0
            y_ref[rows_r, :] = jnp.where(row0, A, A - B)
            y_ref[rows_i, :] = jnp.where(row0, B, Cc)
        else:
            y_ref[rows_r, :] = A - B
            y_ref[rows_i, :] = Cc

    yhi, ylo = _split(y_ref[...])
    ghi = ghi_ref[...]
    y = (jnp.dot(ghi, yhi, preferred_element_type=jnp.float32)
         + jnp.dot(ghi, ylo, preferred_element_type=jnp.float32)
         + jnp.dot(glo_ref[...], yhi, preferred_element_type=jnp.float32))
    kvf = kv.astype(jnp.float32)
    y = y.astype(jnp.bfloat16).astype(jnp.float32) + kvf * d_ref[...].astype(jnp.float32)
    out_a = xn.astype(jnp.float32) * y

    hh = jnp.dot(xn, w1_ref[...], preferred_element_type=jnp.float32)
    hh = hh * jax.nn.sigmoid(hh)
    out_b = jnp.dot(hh.astype(jnp.bfloat16), w2_ref[...], preferred_element_type=jnp.float32)

    o_ref[0] = (x + out_a + out_b).astype(o_ref.dtype)


@jax.jit
def pallas_parallel_sum__ssm_conv_h3__dense_activation_silu__prompt_kernel(
    A_q: jax.Array,
    A_k: jax.Array,
    A_v: jax.Array,
    A_shift_k: jax.Array,
    A_ssm_k: jax.Array,
    A_ssm_D: jax.Array,
    B_x: jax.Array,
    B_w1: jax.Array,
    B_w2: jax.Array,
):
    B, S, D = A_q.shape
    F = B_w1.shape[1]
    ks = A_shift_k.shape[1]
    assert B == 1 and S % C == 0
    N = S // C
    sk_t = A_shift_k.T
    d2 = A_ssm_D.reshape(1, D)

    seq_spec = pl.BlockSpec((1, C, D), lambda a: (0, a, 0))
    return pl.pallas_call(
        _kernel,
        grid=(N,),
        in_specs=[
            seq_spec, seq_spec, seq_spec,
            pl.BlockSpec((ks, D), lambda a: (0, 0)),
            pl.BlockSpec((D, C), lambda a: (0, a)),
            pl.BlockSpec((1, D), lambda a: (0, 0)),
            pl.BlockSpec((D, F), lambda a: (0, 0)),
            pl.BlockSpec((F, D), lambda a: (0, 0)),
        ],
        out_specs=seq_spec,
        out_shape=jax.ShapeDtypeStruct((B, S, D), A_q.dtype),
        scratch_shapes=[
            pltpu.VMEM((2 * C, C), jnp.bfloat16),
            pltpu.VMEM((2 * C, C), jnp.bfloat16),
            pltpu.VMEM((C, 2 * C), jnp.bfloat16),
            pltpu.VMEM((C, 2 * C), jnp.bfloat16),
            pltpu.VMEM((2 * C, D), jnp.float32),
            pltpu.VMEM((C + 8, D), jnp.float32),
            pltpu.VMEM((2 * C, D), jnp.float32),
            pltpu.VMEM((N, 2 * C, D), jnp.float32),
            pltpu.VMEM((N, 2 * C, D), jnp.float32),
            pltpu.VMEM((2 * C, D), jnp.float32),
        ],
        compiler_params=pltpu.CompilerParams(
            dimension_semantics=("arbitrary",),
            vmem_limit_bytes=96 * 1024 * 1024,
        ),
    )(A_q, A_k, A_v, sk_t, A_ssm_k, d2, B_w1, B_w2)
```

```python
import math

import jax
import jax.numpy as jnp
import jax.experimental.pallas as pl
import jax.experimental.pallas.tpu as pltpu

C = 128
RT = 32


def _split(x):
    hi = x.astype(jnp.bfloat16)
    lo = (x - hi.astype(jnp.float32)).astype(jnp.bfloat16)
    return hi, lo


def _dot(a, b):
    return jnp.dot(a, b, preferred_element_type=jnp.float32)


def _kernel(q_ref, k_ref, v_ref, sk_ref, ssmk_ref, d_ref, w1_ref, w2t_ref,
            o_ref,
            fhi_ref, flo_ref, ghi_ref, glo_ref,
            kprev_ref, hprev_ref, uf_ref, kf_ref, y_ref):
    a = pl.program_id(0)
    D = q_ref.shape[1]

    @pl.when(a == 0)
    def _init():
        n = jax.lax.broadcasted_iota(jnp.int32, (C, 2 * C), 0)
        c = jax.lax.broadcasted_iota(jnp.int32, (C, 2 * C), 1)
        f = jnp.where(c > C, c - C, c)
        ang = ((f * n) % (2 * C)).astype(jnp.float32) * (math.pi / C)
        hi, lo = _split(jnp.where(c > C, -jnp.sin(ang), jnp.cos(ang)))
        fhi_ref[...] = hi
        flo_ref[...] = lo
        r = jax.lax.broadcasted_iota(jnp.int32, (2 * C, C), 0)
        b = jax.lax.broadcasted_iota(jnp.int32, (2 * C, C), 1)
        f = jnp.where(r > C, r - C, r)
        ang = ((f * (b + C)) % (2 * C)).astype(jnp.float32) * (math.pi / C)
        scale = jnp.where((r == 0) | (r == C), 0.5 / C, 1.0 / C)
        hi, lo = _split(jnp.where(r > C, -jnp.sin(ang), jnp.cos(ang)) * scale)
        ghi_ref[...] = hi
        glo_ref[...] = lo
        kprev_ref[...] = jnp.zeros(kprev_ref.shape, jnp.float32)
        hprev_ref[...] = jnp.zeros(hprev_ref.shape, jnp.float32)

    x = q_ref[0].astype(jnp.float32)
    mu = jnp.mean(x, axis=0, keepdims=True)
    xc = x - mu
    var = jnp.mean(xc * xc, axis=0, keepdims=True)
    xn = (xc * jax.lax.rsqrt(var + 1e-5)).astype(jnp.bfloat16).astype(jnp.float32)

    kcur = k_ref[0].astype(jnp.float32)
    kprev = kprev_ref[...]
    sk = sk_ref[...].astype(jnp.float32)
    lane = jax.lax.broadcasted_iota(jnp.int32, (D, C), 1)
    ks = kcur * sk[:, 0:1]
    for j in range(1, sk.shape[1]):
        sh = jnp.where(lane < j, pltpu.roll(kprev, j, 1), pltpu.roll(kcur, j, 1))
        ks = ks + sh * sk[:, j:j + 1]
    kprev_ref[...] = kcur
    kv = (ks.astype(jnp.bfloat16).astype(jnp.float32)
          * v_ref[0].astype(jnp.float32)).astype(jnp.bfloat16)

    fhi = fhi_ref[...]
    flo = flo_ref[...]
    h = _dot(kv, fhi) + _dot(kv, flo)
    lane2 = jax.lax.broadcasted_iota(jnp.int32, (D, 2 * C), 1)
    uf_ref[a] = hprev_ref[...] + jnp.where(lane2 % 2 == 0, h, -h)
    hprev_ref[...] = h
    kc = ssmk_ref[...]
    kf_ref[a] = _dot(kc, fhi) + _dot(kc, flo)

    col0 = jax.lax.broadcasted_iota(jnp.int32, (RT, C), 1) == 0
    for rt in range(D // RT):
        rows = pl.ds(rt * RT, RT)

        def body(m, carry):
            A, B, Cc = carry
            kr = kf_ref[m, rows, pl.ds(0, C)]
            ki = kf_ref[m, rows, pl.ds(C, C)]
            ur = uf_ref[a - m, rows, pl.ds(0, C)]
            ui = uf_ref[a - m, rows, pl.ds(C, C)]
            return A + kr * ur, B + ki * ui, Cc + (kr * ui + ki * ur)

        z = jnp.zeros((RT, C), jnp.float32)
        A, B, Cc = jax.lax.fori_loop(0, a + 1, body, (z, z, z))
        y_ref[rows, pl.ds(0, C)] = jnp.where(col0, A, A - B)
        y_ref[rows, pl.ds(C, C)] = jnp.where(col0, B, Cc)

    yhi, ylo = _split(y_ref[...])
    ghi = ghi_ref[...]
    y = _dot(yhi, ghi) + _dot(ylo, ghi) + _dot(yhi, glo_ref[...])
    y = (y.astype(jnp.bfloat16).astype(jnp.float32)
         + kv.astype(jnp.float32) * d_ref[...].astype(jnp.float32))
    out_a = xn * y

    xn_t = xn.T.astype(jnp.bfloat16)
    hh = _dot(xn_t, w1_ref[...])
    hh = hh * jax.nn.sigmoid(hh)
    out_b = jax.lax.dot_general(w2t_ref[...], hh.astype(jnp.bfloat16),
                                (((1,), (1,)), ((), ())),
                                preferred_element_type=jnp.float32)

    o_ref[0] = (x + out_a + out_b).astype(o_ref.dtype)


@jax.jit
def pallas_parallel_sum__ssm_conv_h3__dense_activation_silu__prompt_kernel(
    A_q: jax.Array,
    A_k: jax.Array,
    A_v: jax.Array,
    A_shift_k: jax.Array,
    A_ssm_k: jax.Array,
    A_ssm_D: jax.Array,
    B_x: jax.Array,
    B_w1: jax.Array,
    B_w2: jax.Array,
):
    B, S, D = A_q.shape
    F = B_w1.shape[1]
    ks = A_shift_k.shape[1]
    assert B == 1 and S % C == 0 and D % RT == 0
    N = S // C
    tr = lambda t: jnp.transpose(t, (0, 2, 1))

    seq_spec = pl.BlockSpec((1, D, C), lambda a: (0, 0, a))
    out_t = pl.pallas_call(
        _kernel,
        grid=(N,),
        in_specs=[
            seq_spec, seq_spec, seq_spec,
            pl.BlockSpec((D, ks), lambda a: (0, 0)),
            pl.BlockSpec((D, C), lambda a: (0, a)),
            pl.BlockSpec((D, 1), lambda a: (0, 0)),
            pl.BlockSpec((D, F), lambda a: (0, 0)),
            pl.BlockSpec((D, F), lambda a: (0, 0)),
        ],
        out_specs=seq_spec,
        out_shape=jax.ShapeDtypeStruct((B, D, S), A_q.dtype),
        scratch_shapes=[
            pltpu.VMEM((C, 2 * C), jnp.bfloat16),
            pltpu.VMEM((C, 2 * C), jnp.bfloat16),
            pltpu.VMEM((2 * C, C), jnp.bfloat16),
            pltpu.VMEM((2 * C, C), jnp.bfloat16),
            pltpu.VMEM((D, C), jnp.float32),
            pltpu.VMEM((D, 2 * C), jnp.float32),
            pltpu.VMEM((N, D, 2 * C), jnp.float32),
            pltpu.VMEM((N, D, 2 * C), jnp.float32),
            pltpu.VMEM((D, 2 * C), jnp.float32),
        ],
        compiler_params=pltpu.CompilerParams(
            dimension_semantics=("arbitrary",),
            vmem_limit_bytes=96 * 1024 * 1024,
        ),
    )(tr(A_q), tr(A_k), tr(A_v), A_shift_k, A_ssm_k, A_ssm_D.reshape(D, 1),
      B_w1, B_w2.T)
    return tr(out_t)
```

```python
import math

import jax
import jax.numpy as jnp
import jax.experimental.pallas as pl
import jax.experimental.pallas.tpu as pltpu

C = 128
RT = 16


def _split(x):
    hi = x.astype(jnp.bfloat16)
    lo = (x - hi.astype(jnp.float32)).astype(jnp.bfloat16)
    return hi, lo


def _dot(a, b):
    return jnp.dot(a, b, preferred_element_type=jnp.float32)


def _kernel(q_ref, k_ref, v_ref, sk_ref, ssmk_ref, d_ref, w1_ref, w2t_ref,
            o_ref,
            fhi_ref, flo_ref, ghi_ref, glo_ref,
            kprev_ref, hprev_ref, uf_ref, kf_ref, y_ref, kv_ref, bc_ref):
    a = pl.program_id(0) * 2
    nks = sk_ref.shape[1]
    D = q_ref.shape[1]

    @pl.when(a == 0)
    def _init():
        n = jax.lax.broadcasted_iota(jnp.int32, (C, 2 * C), 0)
        c = jax.lax.broadcasted_iota(jnp.int32, (C, 2 * C), 1)
        f = jnp.where(c > C, c - C, c)
        ang = ((f * n) % (2 * C)).astype(jnp.float32) * (math.pi / C)
        hi, lo = _split(jnp.where(c > C, -jnp.sin(ang), jnp.cos(ang)))
        fhi_ref[...] = hi
        flo_ref[...] = lo
        r = jax.lax.broadcasted_iota(jnp.int32, (2 * C, C), 0)
        b = jax.lax.broadcasted_iota(jnp.int32, (2 * C, C), 1)
        f = jnp.where(r > C, r - C, r)
        ang = ((f * (b + C)) % (2 * C)).astype(jnp.float32) * (math.pi / C)
        scale = jnp.where((r == 0) | (r == C), 0.5 / C, 1.0 / C)
        hi, lo = _split(jnp.where(r > C, -jnp.sin(ang), jnp.cos(ang)) * scale)
        ghi_ref[...] = hi
        glo_ref[...] = lo
        kprev_ref[...] = jnp.zeros(kprev_ref.shape, jnp.float32)
        sk = sk_ref[...].astype(jnp.float32)
        for j in range(nks):
            bc_ref[j] = jnp.broadcast_to(sk[:, j:j + 1], (D, C))
        bc_ref[nks] = jnp.broadcast_to(d_ref[...].astype(jnp.float32), (D, C))
        hprev_ref[...] = jnp.zeros(hprev_ref.shape, jnp.float32)

    x = q_ref[0].astype(jnp.float32)
    mu = jnp.mean(x, axis=0, keepdims=True)
    xc = x - mu
    var = jnp.mean(xc * xc, axis=0, keepdims=True)
    xn = (xc * jax.lax.rsqrt(var + 1e-5)).astype(jnp.bfloat16).astype(jnp.float32)

    lane = jax.lax.broadcasted_iota(jnp.int32, (D, C), 1)
    for hf in range(2):
        cols = pl.ds(hf * C, C)
        kcur = k_ref[0, :, cols].astype(jnp.float32)
        kprev = kprev_ref[...]
        ks = kcur * bc_ref[0]
        for j in range(1, nks):
            sh = jnp.where(lane < j, pltpu.roll(kprev, j, 1), pltpu.roll(kcur, j, 1))
            ks = ks + sh * bc_ref[j]
        kprev_ref[...] = kcur
        kv_ref[:, cols] = (ks.astype(jnp.bfloat16).astype(jnp.float32)
                           * v_ref[0, :, cols].astype(jnp.float32)).astype(jnp.bfloat16)

    fhi = fhi_ref[...]
    flo = flo_ref[...]
    lane2 = jax.lax.broadcasted_iota(jnp.int32, (D, 2 * C), 1)
    for hf in range(2):
        cols = pl.ds(hf * C, C)
        kvh = kv_ref[:, cols]
        h = _dot(kvh, fhi) + _dot(kvh, flo)
        uf_ref[a + hf] = hprev_ref[...] + jnp.where(lane2 % 2 == 0, h, -h)
        hprev_ref[...] = h
        kc = ssmk_ref[:, cols]
        kf_ref[a + hf] = _dot(kc, fhi) + _dot(kc, flo)

    col0 = jax.lax.broadcasted_iota(jnp.int32, (RT, C), 1) == 0
    re, im = pl.ds(0, C), pl.ds(C, C)
    for rt in range(D // RT):
        rows = pl.ds(rt * RT, RT)

        def body(m, carry):
            A0, B0, C0, A1, B1, C1, pr, pi = carry
            kr = kf_ref[m, rows, re]
            ki = kf_ref[m, rows, im]
            ur = uf_ref[a - m, rows, re]
            ui = uf_ref[a - m, rows, im]
            return (A0 + kr * ur, B0 + ki * ui, C0 + (kr * ui + ki * ur),
                    A1 + kr * pr, B1 + ki * pi, C1 + (kr * pi + ki * pr), ur, ui)

        z = jnp.zeros((RT, C), jnp.float32)
        A0, B0, C0, A1, B1, C1, pr, pi = jax.lax.fori_loop(
            0, a + 1, body,
            (z, z, z, z, z, z, uf_ref[a + 1, rows, re], uf_ref[a + 1, rows, im]))
        kr = kf_ref[a + 1, rows, re]
        ki = kf_ref[a + 1, rows, im]
        A1 = A1 + kr * pr
        B1 = B1 + ki * pi
        C1 = C1 + (kr * pi + ki * pr)
        y_ref[0, rows, re] = jnp.where(col0, A0, A0 - B0)
        y_ref[0, rows, im] = jnp.where(col0, B0, C0)
        y_ref[1, rows, re] = jnp.where(col0, A1, A1 - B1)
        y_ref[1, rows, im] = jnp.where(col0, B1, C1)

    ghi = ghi_ref[...]
    glo = glo_ref[...]
    ys = []
    for hf in range(2):
        yhi, ylo = _split(y_ref[hf])
        y = _dot(yhi, ghi) + _dot(ylo, ghi) + _dot(yhi, glo)
        ys.append(y.astype(jnp.bfloat16).astype(jnp.float32)
                  + kv_ref[:, pl.ds(hf * C, C)].astype(jnp.float32) * bc_ref[nks])
    out_a = xn * jnp.concatenate(ys, axis=1)

    xn_t = xn.T.astype(jnp.bfloat16)
    hh = _dot(xn_t, w1_ref[...])
    hh = hh * jax.nn.sigmoid(hh)
    out_b = jax.lax.dot_general(w2t_ref[...], hh.astype(jnp.bfloat16),
                                (((1,), (1,)), ((), ())),
                                preferred_element_type=jnp.float32)

    o_ref[0] = (x + out_a + out_b).astype(o_ref.dtype)


@jax.jit
def pallas_parallel_sum__ssm_conv_h3__dense_activation_silu__prompt_kernel(
    A_q: jax.Array,
    A_k: jax.Array,
    A_v: jax.Array,
    A_shift_k: jax.Array,
    A_ssm_k: jax.Array,
    A_ssm_D: jax.Array,
    B_x: jax.Array,
    B_w1: jax.Array,
    B_w2: jax.Array,
):
    B, S, D = A_q.shape
    F = B_w1.shape[1]
    ks = A_shift_k.shape[1]
    assert B == 1 and S % (2 * C) == 0 and D % RT == 0
    N = S // C
    tr = lambda t: jnp.transpose(t, (0, 2, 1))

    seq_spec = pl.BlockSpec((1, D, 2 * C), lambda a: (0, 0, a))
    out_t = pl.pallas_call(
        _kernel,
        grid=(N // 2,),
        in_specs=[
            seq_spec, seq_spec, seq_spec,
            pl.BlockSpec((D, ks), lambda a: (0, 0)),
            pl.BlockSpec((D, 2 * C), lambda a: (0, a)),
            pl.BlockSpec((D, 1), lambda a: (0, 0)),
            pl.BlockSpec((D, F), lambda a: (0, 0)),
            pl.BlockSpec((D, F), lambda a: (0, 0)),
        ],
        out_specs=seq_spec,
        out_shape=jax.ShapeDtypeStruct((B, D, S), A_q.dtype),
        scratch_shapes=[
            pltpu.VMEM((C, 2 * C), jnp.bfloat16),
            pltpu.VMEM((C, 2 * C), jnp.bfloat16),
            pltpu.VMEM((2 * C, C), jnp.bfloat16),
            pltpu.VMEM((2 * C, C), jnp.bfloat16),
            pltpu.VMEM((D, C), jnp.float32),
            pltpu.VMEM((D, 2 * C), jnp.float32),
            pltpu.VMEM((N, D, 2 * C), jnp.float32),
            pltpu.VMEM((N, D, 2 * C), jnp.float32),
            pltpu.VMEM((2, D, 2 * C), jnp.float32),
            pltpu.VMEM((D, 2 * C), jnp.bfloat16),
            pltpu.VMEM((ks + 1, D, C), jnp.float32),
        ],
        compiler_params=pltpu.CompilerParams(
            dimension_semantics=("arbitrary",),
            vmem_limit_bytes=96 * 1024 * 1024,
        ),
    )(tr(A_q), tr(A_k), tr(A_v), A_shift_k, A_ssm_k, A_ssm_D.reshape(D, 1),
      B_w1, B_w2.T)
    return tr(out_t)
```
